```python
import os as _os
_os.environ.setdefault("JAX_PLATFORMS", "cpu")
import jax
import jax.numpy as jnp

def _softmax(x, axis=-1):
    return jax.nn.softmax(x, axis=axis)
def _gelu(x):
    return jax.nn.gelu(x, approximate=True)
def _silu(x):
    return jax.nn.silu(x)
def _sigmoid(x):
    return jax.nn.sigmoid(x)
def _layernorm(x, axis=-1, eps=1e-5):
    m = jnp.mean(x, axis=axis, keepdims=True)
    v = jnp.var(x, axis=axis, keepdims=True)
    return (x - m) / jnp.sqrt(v + eps)
def _scatter_add(tgt, idx, src, axis=0):
    return tgt.at[idx].add(src)
def _segment_sum(src, seg, n):
    return jax.ops.segment_sum(src, seg, n)
class _Rng:
    def __init__(self, key):
        self._k = key
    def _next(self):
        self._k, sub = jax.random.split(self._k)
        return sub
    def normal(self, shape):
        return jax.random.normal(self._next(), shape, dtype=jnp.bfloat16)
    def randint(self, lo, hi, shape):
        return jax.random.randint(self._next(), shape, lo, hi, dtype=jnp.int32)
    def uniform(self, shape, lo=0.0, hi=1.0):
        return jax.random.uniform(self._next(), shape, jnp.bfloat16, lo, hi)
    def permutation(self, n):
        return jax.random.permutation(self._next(), n)


kernel_name = 'standalone__fft_conv__vision'

def setup_inputs():
    _rng = _Rng(jax.random.key(int.from_bytes(__import__("os").urandom(4), "little")))
    _w = (lambda a: (lambda t: t.astype(jnp.bfloat16) if jnp.issubdtype(t.dtype, jnp.floating) else t)(jnp.asarray(a)))
    H = W = 224
    C = 96
    K = 3
    return {
        "x": _w((lambda *s: _rng.normal(s) * 0.05)(1, H, W, C)),
        "w": _w((lambda *s: _rng.normal(s) * 0.05)(K, K, C, C)),
    }

def reference(x, w):
    B, H, W, C = x.shape
    K = w.shape[0]
    wp = jnp.pad(w, ((0, H - K), (0, W - K), (0, 0), (0, 0)))
    Xf = (lambda x, axes=(-2,-1): jnp.fft.rfft2(x.astype(jnp.float32), axes=axes))(x, axes=(1, 2))
    Wf = (lambda x, axes=(-2,-1): jnp.fft.rfft2(x.astype(jnp.float32), axes=axes))(wp, axes=(0, 1))
    Yf = jnp.einsum('bhwi,hwio->bhwo', Xf, Wf)
    y = (lambda x, s, axes=(-2,-1): jnp.fft.irfft2(x, s=s, axes=axes).astype(jnp.bfloat16))(Yf, (H, W), axes=(1, 2))
    return y
```

```python
import functools
import numpy as np, jax, jax.numpy as jnp
from jax import lax
from jax.experimental import pallas as pl
from jax.experimental.pallas import tpu as pltpu
H = W = 224; C = 96; CH = C // 2
NSET = 4; HS = H // NSET
f32 = jnp.float32; bf16 = jnp.bfloat16; i32 = jnp.int32
tb = lambda v: pltpu.bitcast(v, bf16)
ti = lambda v: pltpu.bitcast(v, i32)

def lagr(pts):
    G = []
    for i, p in enumerate(pts):
        n = np.prod([p - q for j, q in enumerate(pts) if j != i])
        G.append(np.array([1.0, p, p * p]) / n)
    G.append(np.array([0.0, 0.0, 1.0]))
    return np.array(G)

class F2:
    m = 2
    G = np.array([[.5, .5, .5], [.5, -.5, .5], [1, 0, 0], [0, 0, 1]])
    @staticmethod
    def bt(d): return [d[1] + d[2], d[2] - d[1], d[0] - d[2], d[3] - d[1]]
    @staticmethod
    def at(m): return [(m[0] + m[1]) + m[2], (m[0] - m[1]) + m[3]]

class F3:
    m = 3
    a = 0.4
    G = lagr([a, -a, 1.0, -1.0])
    @classmethod
    def bt(c, d):
        a = c.a
        p = d[3] - d[1]; q = (d[2] - d[0]) * a
        p2 = d[3] - d[1] * (a * a); q2 = d[2] - d[0] * (a * a)
        return [p + q, p - q, p2 + q2, p2 - q2, (d[4] - d[2]) - q * a]
    @classmethod
    def at(c, m):
        a = c.a
        s1, t1, s2, t2 = m[0] + m[1], m[0] - m[1], m[2] + m[3], m[2] - m[3]
        return [s1 + s2, t1 * a + t2, (s1 * (a * a) + s2) + m[4]]

class F4:
    m = 4
    a, b = 2 / 3, 1.5
    G = lagr([a, -a, b, -b, 0.0])
    @classmethod
    def bt(c, d):
        a, b = c.a, c.b
        a2d2 = d[2] * (a * a)
        p = d[4] - d[2] * (b * b); q = d[3] * a - d[1] * b
        p2 = d[4] - a2d2; q2 = d[3] * b - d[1] * a
        return [p + q, p - q, p2 + q2, p2 - q2, d[0] + p - a2d2, d[1] + d[5] - d[3] * (a * a + b * b)]
    @classmethod
    def at(c, m):
        a, b = c.a, c.b
        s1, t1, s2, t2 = m[0] + m[1], m[0] - m[1], m[2] + m[3], m[2] - m[3]
        return [s1 + s2 + m[4], t1 * a + t2 * b, s1 * (a * a) + s2 * (b * b), t1 * a**3 + t2 * b**3 + m[5]]

def spread(lo, hi, *rest):
    n = 12
    if rest: return [lo, hi, *rest]
    return [int(round(lo + i * (hi - lo) / (n - 1))) for i in range(n)]

def make(parts=(F3, F2, F2), rd=(2, 2, 4, 8, 10, 1), wr=(14, 7, 3, 2, 1, 1), dma=True, ref=2, unroll=1, flags=None,
         zstage=True, pc=(1, 12), ub=(8, 41), ud=(8, 41), tie=True):
    NS = HS // 2
    rstart = np.cumsum((0,) + tuple(rd)); wstart = np.cumsum((0,) + tuple(wr))
    assert rstart[-1] == NS - 1 and wstart[-1] == NS
    algs = list(dict.fromkeys(parts))
    goff = {a: int(sum(len(b.G) for b in algs[:i])) for i, a in enumerate(algs)}
    NG = sum(len(a.G) for a in algs)
    coff = [int(v) for v in np.cumsum([0] + [len(a.G) for a in parts])]; poff = [int(v) for v in np.cumsum([0] + [a.m for a in parts])]
    assert poff[-1] == 7
    NC = coff[-1]; NP = len(parts); NU = 12
    wpc, wub, wud = spread(*pc), spread(*ub), spread(*ud)
    G0 = HS * CH

    def kernel(x_hbm, w_ref, o_hbm, xb, ob, gm, wb, yb, zb, cb, db, isem, osem):
        RS = 2 * CH
        x_hbm = x_hbm.bitcast(i32); o_hbm = o_hbm.bitcast(i32)
        gmi = gm.bitcast(i32); ybi = yb.bitcast(i32)
        def rcopy(lo, n, s): return pltpu.make_async_copy(x_hbm.at[:, pl.ds(lo * RS, n * RS)], xb.at[:, pl.ds(lo * RS, n * RS)], isem.at[s])
        halo = lambda: rcopy(NS - 1, 1, len(rd))
        ins = lambda i: rcopy(int(rstart[i]), rd[i], i)
        outs = lambda i: pltpu.make_async_copy(ob.at[:, pl.ds(int(wstart[i]) * RS, wr[i] * RS)], o_hbm.at[:, pl.ds(int(wstart[i]) * RS, wr[i] * RS)], osem.at[i])
        if dma:
            halo().start()
            for i in range(len(rd)): ins(i).start()
        eye = (lax.broadcasted_iota(i32, (C, C), 0) == lax.broadcasted_iota(i32, (C, C), 1)).astype(bf16)
        nt = (((1,), (1,)), ((), ()))
        zpad = jnp.zeros((128 - C, C), bf16)
        g = [[lax.dot_general(eye, jnp.concatenate([w_ref[2 - a, 2 - b], zpad], axis=0), nt, preferred_element_type=f32) for b in range(3)] for a in range(3)]
        def comb(coef, vals):
            acc = None
            for cf, v in zip(coef, vals):
                if cf == 0: continue
                t = v if cf == 1 else v * float(cf)
                acc = t if acc is None else acc + t
            return acc
        for i in range(4):
            gh = [comb(F2.G[i], [g[a][b] for a in range(3)]) for b in range(3)]
            for alg in algs:
                for j in range(len(alg.G)):
                    gm[goff[alg] + j, i] = comb(alg.G[j], gh).astype(bf16)
                    if tie: ob[i, pl.ds(G0 + (goff[alg] + j) * CH, CH), pl.ds(0, 128)] = gmi[goff[alg] + j, i]

        lane = lax.broadcasted_iota(i32, (8, 128), 1)
        e = lane % 7
        bits = [(e & (1 << k)) != 0 for k in range(3)]
        wrap = (lane & 31) == ref
        mo = lambda t: t * RS if isinstance(t, int) else pl.multiple_of(t * RS, RS)
        rot = lambda v, s: v if s % 128 == 0 else pltpu.roll(v, s % 128, 1)
        st = {}

        def pa(t, n, sh=0):
            rows = pl.ds(mo(t) + 8 * n, 8)
            B = [xb[(r - sh) % 4, rows, pl.ds(128, 96)] for r in range(4)]
            for r in range(3):
                cb[r, pl.ds(8 * n, 8), :] = jnp.concatenate([B[r][:, :96 - 32 * r], B[r + 1][:, 64 - 32 * r:]], axis=1)

        def px(t, slot, n, sh=0):
            rows = pl.ds(mo(t) + 8 * n, 8)
            c = [cb[r, pl.ds(8 * n, 8), :] for r in range(3)]
            A = [xb[(r - sh) % 4, rows, pl.ds(0, 128)] for r in range(4)]
            v = [A[0], c[0], A[1], c[1], A[2], c[2], A[3]]
            S = [v[(4 * q) % 7] for q in range(7)]
            for k in range(3):
                S = [jnp.where(bits[k], S[(j - (1 << k)) % 7], S[j]) for j in range(7)]
            V = [jnp.where(wrap, rot(S[k % 7], ref - k - W), rot(S[k % 7], ref - k)) for k in (-2, -1)] + [rot(S[k], ref - k) for k in range(7)]
            d = [tb(u).astype(f32) for u in V]
            for ip, alg in enumerate(parts):
                for j, u in enumerate(alg.bt(d[poff[ip]:poff[ip] + alg.m + 2])):
                    wb[slot, coff[ip] + j, pl.ds(16 * n, 16), :] = u

        def mm(sp, sc, ip, j, hook):
            c = coff[ip] + j; gi = goff[parts[ip]] + j
            r = F2.bt([wb[s, c, pl.ds(o, C), :] for s in (sp, sc) for o in (0, C)])
            L = [[] for _ in range(4)]
            for q in range(6):
                for i in range(4):
                    L[i].append(ob[i, pl.ds(G0 + gi * CH + 8 * q, 8), pl.ds(0, 128)] if tie else gmi[gi, i, pl.ds(8 * q, 8), :])
                hook(6 * c + q)
            m = [jnp.dot(tb(jnp.concatenate(L[i], axis=0))[:, :C], v.astype(bf16), preferred_element_type=f32) for i, v in enumerate(r)]
            return F2.at(m)

        def f_ua(n):
            st[n] = [rot(ybi[k, pl.ds(8 * n, 8), :], k - ref) for k in range(7)]

        def f_ub(t, n):
            S = st.pop(n)
            for k in range(3):
                S = [jnp.where(bits[k], S[(j + (1 << k)) % 7], S[j]) for j in range(7)]
            v = [S[(2 * q) % 7] for q in range(7)]
            rows = pl.ds(mo(t) + 8 * n, 8)
            for r in range(4): ob[r, rows, pl.ds(0, 128)] = v[2 * r]
            ob[0, rows, pl.ds(128, 96)] = v[1][:, :96]
            for r in range(3): db[r, pl.ds(8 * n, 8), :] = v[2 * r + 1]

        def f_ud(t, n):
            v = [db[r, pl.ds(8 * n, 8), :] for r in range(3)]; r = [rot(u, -32) for u in v]
            rows = pl.ds(mo(t) + 8 * n, 8)
            ob[1, rows, pl.ds(128, 96)] = jnp.where(lane < 64, v[1], r[0])[:, :96]
            ob[2, rows, pl.ds(128, 96)] = jnp.where(lane < 32, v[2], r[1])[:, :96]
            ob[3, rows, pl.ds(128, 96)] = r[2][:, :96]

        yb[...] = jnp.zeros(yb.shape, bf16)
        db[...] = jnp.zeros(db.shape, i32)
        if dma: halo().wait()
        for n in range(NU): pa(NS - 1, n, 1)
        for n in range(NU): px(NS - 1, 0, n, 1)
        if dma: ins(0).wait()
        for n in range(NU): pa(0, n)
        for n in range(NU): px(0, 1, n)
        for n in range(NU): pa(1, n)

        def step(t, sp, sc, sn, ys, z0):
            tp, tn = jnp.maximum(t - 1, 0), jnp.minimum(t + 1, NS - 1)
            def hook(p):
                for n in range(NU):
                    if wud[n] == p: f_ud(jnp.maximum(t - 2, 0), n)
                    if wub[n] == p: f_ub(tp, n)
            for n in range(NU): f_ua(n)
            c = 0
            pend = []
            for ip, alg in enumerate(parts):
                z = []
                nj = len(alg.G)
                keep = 2 if alg is F2 else nj - 1
                for j in range(nj):
                    zz = mm(sp, sc, ip, j, hook)
                    if zstage and j < keep:
                        for u in range(2): zb[0, c, u] = zz[u]
                    z.append(zz)
                    if zstage and j == nj - 1:
                        z[:keep] = [[zb[z0, coff[ip] + jj, u] for u in range(2)] for jj in range(keep)]
                    for n in range(NU):
                        if min(wpc[n], NC - 1) == c: px(tn, sn, n)
                    c += 1
                for u in range(2):
                    for k, y in enumerate(alg.at([zz[u] for zz in z])):
                        yb[poff[ip] + k, pl.ds(u * C, C), :] = y.astype(bf16)
            for n in range(NU): pa(jnp.minimum(t + 2, NS - 1), n)

        def body(u, sp):
            t = u * unroll
            if dma:
                for i in range(1, len(rd)):
                    @pl.when(u == (int(rstart[i]) - 2) // unroll)
                    def _():
                        ins(i).wait()
                for i in range(len(wr)):
                    s = -(-(int(wstart[i + 1]) + 2) // unroll)
                    if s < NS // unroll:
                        @pl.when(u == s)
                        def _():
                            outs(i).start()
            for k in range(unroll):
                sc = jnp.where(sp == 2, 0, sp + 1); sn = jnp.where(sc == 2, 0, sc + 1)
                step(t + k, sp, sc, sn, (t & 1) if unroll == 1 else k % 2, sp >> 2)
                sp = sc
            return sp
        lax.fori_loop(0, NS // unroll, body, 0)
        for n in range(NU): f_ud(NS - 2, n)
        if dma:
            for i in range(len(wr) - 1):
                if -(-(int(wstart[i + 1]) + 2) // unroll) >= NS // unroll: outs(i).start()
        for n in range(NU): f_ua(n)
        for n in range(NU): f_ub(NS - 1, n)
        for n in range(NU): f_ud(NS - 1, n)
        if dma:
            outs(len(wr) - 1).start()
            for i in range(len(wr)): outs(i).wait()

    def f(x, w):
        xt = jnp.transpose(x, (0, 1, 3, 2)).reshape(NSET, HS * C, W)
        y = pl.pallas_call(kernel,
            in_specs=[pl.BlockSpec(memory_space=pl.ANY), pl.BlockSpec(memory_space=pltpu.VMEM)],
            out_specs=pl.BlockSpec(memory_space=pl.ANY),
            out_shape=jax.ShapeDtypeStruct((NSET, HS * C, W), bf16),
            scratch_shapes=[pltpu.VMEM((NSET, HS * CH, W), i32), pltpu.VMEM((NSET, (HS + NG) * CH, W), i32),
                            pltpu.VMEM((NG, 4, C, 128), bf16),
                            pltpu.VMEM((3, NC, 2 * C, 128), f32), pltpu.VMEM((7, 2 * C, 128), bf16), pltpu.VMEM((2, NC, 2, C, 128), f32), pltpu.VMEM((3, 2 * CH, 128), i32), pltpu.VMEM((3, 2 * CH, 128), i32),
                            pltpu.SemaphoreType.DMA((len(rd) + 1,)), pltpu.SemaphoreType.DMA((len(wr),))],
            compiler_params=pltpu.CompilerParams(vmem_limit_bytes=100 * 2**20, flags=flags),
        )(xt, w)
        return jnp.transpose(y.reshape(1, H, C, W), (0, 1, 3, 2))
    return f


@jax.jit
def pallas_standalone__fft_conv__vision_kernel(x, w):
    return make(pc=(8, 14), ub=(8, 35), ud=(8, 20), parts=(F4, F3), wr=(10, 6, 4, 3, 2, 1, 1, 1))(x, w)
```

```python
import jax
import jax.numpy as jnp
import numpy as np
from jax import lax
import jax.experimental.pallas as pl
import jax.experimental.pallas.tpu as pltpu

H = W = 224
C = 96
LO, HI = 128, W - 128
NSET = 4
NSTEP = H // NSET // 2
NPHASE = 7
NUNIT = 2 * C // 16

f32, bf16, i32 = jnp.float32, jnp.bfloat16, jnp.int32


def _filter_matrix(points):
    rows = []
    for i, p in enumerate(points):
        norm = np.prod([p - q for j, q in enumerate(points) if j != i])
        rows.append(np.array([1.0, p, p * p]) / norm)
    return np.array(rows + [np.array([0.0, 0.0, 1.0])])


def _f2_bt(d):
    return [d[1] + d[2], d[2] - d[1], d[0] - d[2], d[3] - d[1]]


def _f2_at(m):
    return [(m[0] + m[1]) + m[2], (m[0] - m[1]) + m[3]]


_A3 = 0.4


def _f3_bt(d):
    a = _A3
    p, q = d[3] - d[1], (d[2] - d[0]) * a
    p2, q2 = d[3] - d[1] * (a * a), d[2] - d[0] * (a * a)
    return [p + q, p - q, p2 + q2, p2 - q2, (d[4] - d[2]) - q * a]


def _f3_at(m):
    a = _A3
    s1, t1, s2, t2 = m[0] + m[1], m[0] - m[1], m[2] + m[3], m[2] - m[3]
    return [s1 + s2, t1 * a + t2, (s1 * (a * a) + s2) + m[4]]


_A4, _B4 = 2 / 3, 1.5


def _f4_bt(d):
    a, b = _A4, _B4
    a2d2 = d[2] * (a * a)
    p, q = d[4] - d[2] * (b * b), d[3] * a - d[1] * b
    p2, q2 = d[4] - a2d2, d[3] * b - d[1] * a
    return [p + q, p - q, p2 + q2, p2 - q2,
            d[0] + p - a2d2, d[1] + d[5] - d[3] * (a * a + b * b)]


def _f4_at(m):
    a, b = _A4, _B4
    s1, t1, s2, t2 = m[0] + m[1], m[0] - m[1], m[2] + m[3], m[2] - m[3]
    return [s1 + s2 + m[4], t1 * a + t2 * b,
            s1 * (a * a) + s2 * (b * b), t1 * a**3 + t2 * b**3 + m[5]]


W_TILES = (
    (0, 4, 0, _filter_matrix([_A4, -_A4, _B4, -_B4, 0.0]), _f4_bt, _f4_at, (0, 1, 4, 5, 2, 3), 3),
    (4, 3, 6, _filter_matrix([_A3, -_A3, 1.0, -1.0]), _f3_bt, _f3_at, (0, 1, 4, 2, 3), 3),
)
NCOMP = 11

SPLIT_ROUND = (6, 6, 7, 9, 10, 10, 10, 10, 10, 10, 10, 10)
MERGE_SLOT = (7, 9, 11, 13, 15, 17, 18, 20, 22, 24, 26, 28)
UNSTRIP_SLOT = (6, 8, 10, 12, 14, 16, 18, 20, 22, 24, 26, 28)
READS_PER_STEP = 3
ORDERED_READS = 18
PROLOGUE_READS = (9, 2, 3, 1, 3, 6)
PHASES = ((10, 2, 0), (1, 0, 0), (10, 0, 2), (5, 0, 1))
PARK_PAD = 8


def _kernel(x_hbm, w_hbm, y_hbm, x_lo, x_hi, y_lo, y_hi, w_vmem, pack, y_poly, park,
            x_seam, y_seam, read_sem, write_sem, *x_wino):
    x_lo32, x_hi32, y_lo32, y_hi32, pack32, y_poly32 = (
        r.bitcast(i32) for r in (x_lo, x_hi, y_lo, y_hi, pack, y_poly))

    tile_lanes = (pl.ds(0, LO), pl.ds(LO, HI))

    def read(hi, r, t, rows):
        return pltpu.make_async_copy(x_hbm.at[r, t, rows, tile_lanes[hi]],
                                     (x_lo, x_hi)[hi].at[r, t, rows], read_sem.at[hi * NSTEP + t])

    def start_read(piece, dt=0):
        t = (piece // READS_PER_STEP - 1) % NSTEP + dt
        size = 2 * C // READS_PER_STEP
        for r in range(NSET):
            for hi in range(2):
                read(hi, r, t, pl.ds(piece % READS_PER_STEP * size, size)).start(
                    priority=r % 2 if piece >= ORDERED_READS else 0)

    def prologue_reads(i):
        for piece in range(sum(PROLOGUE_READS[:i]), sum(PROLOGUE_READS[:i + 1])):
            start_read(piece)

    def wait_read(t):
        for hi in range(2):
            read(hi, slice(None), t, slice(None)).wait()

    def write(hi, r, t, rows):
        return pltpu.make_async_copy((y_lo, y_hi)[hi].at[r, t, rows],
                                     y_hbm.at[r, t, rows, tile_lanes[hi]], write_sem.at[hi])

    def start_write(t, halves=(0, 1), merged=True, unstripped=True):
        for u in halves:
            for r in range(NSET):
                for hi in range(2):
                    if unstripped if hi and r else merged:
                        write(hi, r, t, pl.ds(u * C, C)).start()

    def weight_view(i, comp, q):
        return (y_lo32, y_hi32)[i % 2], (i, NSTEP + comp, pl.ds(8 * q, 8), pl.ds(0, C))

    def transform_weights():
        eye = (lax.broadcasted_iota(i32, (C, C), 0)
               == lax.broadcasted_iota(i32, (C, C), 1)).astype(bf16)
        zeros = jnp.zeros((128 - C, C), bf16)
        g = [[lax.dot_general(eye, jnp.concatenate([w_vmem[2 - a, 2 - b], zeros], axis=0),
                              (((1,), (1,)), ((), ())), preferred_element_type=f32)
              for b in range(3)] for a in range(3)]

        def scale(v, coef):
            return v if abs(coef - 1) < 1e-12 else v * float(coef)

        for q in range(C // 16):
            g0, g1, g2 = ([v[16 * q:16 * q + 16] for v in row] for row in g)
            ends = [u + v for u, v in zip(g0, g2)]
            along_h = (([u + v for u, v in zip(ends, g1)], 0.5),
                       ([u - v for u, v in zip(ends, g1)], 0.5), (g0, 1.0), (g2, 1.0))
            for i, (h, factor) in enumerate(along_h):
                for _, _, comp0, gmat, *_ in W_TILES:
                    gmat = gmat * factor
                    out = []
                    for j in (0, 2):
                        even = scale(h[0], gmat[j, 0]) + scale(h[2], gmat[j, 2])
                        odd = scale(h[1], gmat[j, 1])
                        same_sign = gmat[j, 0] * gmat[j + 1, 0] > 0
                        out += [even + odd, even - odd if same_sign else odd - even]
                    for row in gmat[4:]:
                        b = int(np.argmax(np.abs(row)))
                        out.append(scale(h[b], row[b]))
                    for j, v in enumerate(out):
                        pack[comp0 + j, i, pl.ds(16 * q, 16), :] = v.astype(bf16)
                        ref, idx = weight_view(i, comp0 + j, q)
                        ref[idx] = pack32[comp0 + j, i, pl.ds(8 * q, 8), pl.ds(0, C)]

    lane = lax.broadcasted_iota(i32, (8, 128), 1)
    lane_bits = [((lane % NPHASE) & (1 << k)) != 0 for k in range(3)]
    row_start = (lane & 31) == 0

    def rot(v, shift):
        return v if shift % 128 == 0 else pltpu.roll(v, shift % 128, 1)

    def barrel(vs, sign):
        for k in range(3):
            vs = [jnp.where(lane_bits[k], vs[(j + sign * (1 << k)) % NPHASE], vs[j])
                  for j in range(NPHASE)]
        return vs

    def strip(t, n, up=0):
        rows = pl.ds(8 * n, 8)
        hi = [x_hi32[(r - up) % NSET, t, rows, :] for r in range(NSET)]
        for r in range(NSET - 1):
            x_seam[r, rows, :] = jnp.concatenate(
                [hi[r][:, :HI - 32 * r], hi[r + 1][:, 64 - 32 * r:]], axis=1)

    def split(t, slot, n, up=0):
        rows = pl.ds(8 * n, 8)
        seam = [x_seam[r, rows, :] for r in range(NSET - 1)]
        lo = [x_lo32[(r - up) % NSET, t, rows, :] for r in range(NSET)]
        v = [lo[0], seam[0], lo[1], seam[1], lo[2], seam[2], lo[3]]
        s = barrel([v[4 * q % NPHASE] for q in range(NPHASE)], -1)
        ph = [jnp.where(row_start, rot(s[k], -k - W), rot(s[k], -k)) for k in (-2, -1)]
        ph += [rot(s[k], -k) for k in range(NPHASE)]
        d = [pltpu.bitcast(u, bf16).astype(f32) for u in ph]
        for phase0, width, comp0, _, bt, *_ in W_TILES:
            for j, u in enumerate(bt(d[phase0:phase0 + width + 2])):
                x_wino[comp0 + j][slot, pl.ds(16 * n, 16), :] = u

    def align(n):
        return [rot(y_poly32[k, pl.ds(8 * n, 8), :], k) for k in range(NPHASE)]

    def merge(t, n, aligned):
        s = barrel(aligned, 1)
        v = [s[2 * q % NPHASE] for q in range(NPHASE)]
        rows = pl.ds(8 * n, 8)
        for r in range(NSET):
            y_lo32[r, t, rows, :] = v[2 * r]
        y_hi32[0, t, rows, :] = v[1][:, :HI]
        for r in range(NSET - 1):
            y_seam[r, rows, :] = v[2 * r + 1]

    def unstrip(t, n):
        rows = pl.ds(8 * n, 8)
        v = [y_seam[r, rows, :] for r in range(NSET - 1)]
        head = [rot(u, -32) for u in v]
        y_hi32[1, t, rows, :] = jnp.where(lane < 64, v[1], head[0])[:, :HI]
        y_hi32[2, t, rows, :] = jnp.where(lane < 32, v[2], head[1])[:, :HI]
        y_hi32[3, t, rows, :] = head[2][:, :HI]

    def products(tile, prev, cur, zero, at_slot=lambda p: None, after_round=lambda c: None):
        phase0, _, comp0, _, _, at, order, parked = W_TILES[tile]
        z = [None] * len(order)
        for pos, j in enumerate(order):
            comp = comp0 + j
            rhs = _f2_bt([x_wino[comp][s, pl.ds(o, C), :] for s in (prev, cur) for o in (0, C)])
            lhs = [[] for _ in rhs]
            for q in range(C // 16):
                for i in range(4):
                    ref, idx = weight_view(i, comp, q)
                    lhs[i].append(ref[idx])
                at_slot(6 * (comp0 + pos) + q)
            z[j] = _f2_at([jnp.dot(pltpu.bitcast(jnp.concatenate(a, axis=0), bf16),
                                   b.astype(bf16), preferred_element_type=f32)
                           for a, b in zip(lhs, rhs)])
            if pos < parked:
                for u in range(2):
                    park[0, comp, pl.ds(u * C, C), :] = z[j][u]
            after_round(comp0 + pos)
        for j in order[:parked]:
            z[j] = [park[zero, comp0 + j, pl.ds(u * C, C), :] for u in range(2)]
        for u in range(2):
            for k, y in enumerate(at([rows[u] for rows in z])):
                y_poly[phase0 + k, pl.ds(u * C, C), :] = y.astype(bf16)

    def output_work(t):
        aligned = [align(n) for n in range(NUNIT)]

        def at_slot(p):
            for n in range(NUNIT):
                if UNSTRIP_SLOT[n] == p:
                    unstrip(jnp.maximum(t - 2, 0), n)
                if MERGE_SLOT[n] == p:
                    merge(t - 1, n, aligned[n])
        return at_slot

    def step(t, prev):
        cur = jnp.where(prev == 2, 0, prev + 1)
        nxt = jnp.where(cur == 2, 0, cur + 1)
        at_slot = output_work(t)

        def after_round(c):
            for n in range(NUNIT):
                if SPLIT_ROUND[n] == c:
                    split(t + 1, nxt, n)
        for tile in range(len(W_TILES)):
            products(tile, prev, cur, prev >> 2, at_slot, after_round)
        for n in range(NUNIT):
            strip(jnp.minimum(t + 2, NSTEP - 1), n)
        return cur

    def all_units(fn, *args, **kwargs):
        for n in range(NUNIT):
            fn(*args, n, **kwargs)

    w_copy = pltpu.make_async_copy(w_hbm, w_vmem, read_sem.at[2 * NSTEP])
    w_copy.start()
    prologue_reads(0)
    y_seam[...] = jnp.zeros(y_seam.shape, i32)
    w_copy.wait()
    transform_weights()
    prologue_reads(1)
    wait_read(NSTEP - 1)
    all_units(strip, NSTEP - 1, up=1)
    all_units(split, NSTEP - 1, 0, up=1)
    prologue_reads(2)
    wait_read(0)
    all_units(strip, 0)
    all_units(split, 0, 1)
    prologue_reads(3)
    wait_read(1)
    all_units(strip, 1)
    products(0, 0, 1, 0)
    prologue_reads(4)
    wait_read(2)
    all_units(split, 1, 2)
    products(1, 0, 1, 0)
    all_units(strip, 2)
    prologue_reads(5)

    prev, t0, pieces, written = 1, 1, sum(PROLOGUE_READS), 0
    for steps, n_read, n_write in PHASES:
        def body(t, prev):
            if t0 + steps + 1 < NSTEP - 1:
                wait_read(t + 2)
            else:
                pl.when(t + 2 < NSTEP - 1)(lambda: wait_read(t + 2))
            prev = step(t, prev)
            for k in range(n_read * READS_PER_STEP):
                start_read(pieces + k, n_read * (t - t0))
            for k in range(n_write):
                start_write(written + k + n_write * (t - t0))
            return prev
        prev = lax.fori_loop(t0, t0 + steps, body, prev)
        t0 += steps
        pieces += steps * n_read * READS_PER_STEP
        written += steps * n_write
        assert written <= t0 - 2
    assert (t0, pieces, written) == (NSTEP - 1, NSTEP * READS_PER_STEP, NSTEP - 3)

    last, zero = NSTEP - 1, prev >> 2
    start_write(last - 2, unstripped=False)
    products(0, last % 3, NSTEP % 3, zero, output_work(last + zero))
    start_write(last - 2, merged=False)
    start_write(last - 1, unstripped=False)
    all_units(unstrip, last - 1)
    products(1, last % 3, NSTEP % 3, zero)
    start_write(last - 1, merged=False)
    for u in range(2):
        units = range(u * NUNIT // 2, (u + 1) * NUNIT // 2)
        aligned = [align(n) for n in units]
        for n, a in zip(units, aligned):
            merge(last, n, a)
        for n in units:
            unstrip(last, n)
        start_write(last, halves=(u,))
    for hi in range(2):
        write(hi, slice(None), pl.ds(0, NSTEP), slice(None)).wait()


@jax.jit
def pallas_standalone__fft_conv__vision_kernel(x: jax.Array, w: jax.Array):
    assert x.shape == (1, H, W, C) and w.shape == (3, 3, C, C)
    rows = (NSET, NSTEP, 2 * C, W)
    y = pl.pallas_call(
        _kernel,
        in_specs=[pl.BlockSpec(memory_space=pl.ANY), pl.BlockSpec(memory_space=pl.ANY)],
        out_specs=pl.BlockSpec(memory_space=pl.ANY),
        out_shape=jax.ShapeDtypeStruct(rows, bf16),
        scratch_shapes=[
            pltpu.VMEM((NSET, NSTEP, 2 * C, LO), bf16),
            pltpu.VMEM((NSET, NSTEP, 2 * C, HI), bf16),
            pltpu.VMEM((NSET, NSTEP + NCOMP, 2 * C, LO), bf16),
            pltpu.VMEM((NSET, NSTEP + NCOMP, 2 * C, HI), bf16),
            pltpu.VMEM((3, 3, C, C), bf16),
            pltpu.VMEM((NCOMP, 4, C, 128), bf16),
            pltpu.VMEM((NPHASE, 2 * C, 128), bf16),
            pltpu.VMEM((2, NCOMP, 2 * C + PARK_PAD, 128), f32),
            pltpu.VMEM((NSET - 1, C, 128), i32),
            pltpu.VMEM((NSET - 1, C, 128), i32),
            pltpu.SemaphoreType.DMA((2 * NSTEP + 1,)),
            pltpu.SemaphoreType.DMA((2,)),
        ] + [pltpu.VMEM((3, 2 * C, 128), f32)] * NCOMP,
        compiler_params=pltpu.CompilerParams(
            vmem_limit_bytes=100 * 2**20, disable_semaphore_checks=True),
    )(jnp.transpose(x, (0, 1, 3, 2)).reshape(rows), w)
    return jnp.transpose(y.reshape(1, H, C, W), (0, 1, 3, 2))
```
